```python
import jax
import jax.numpy as jnp

def _softmax(x, axis=-1):
    return jax.nn.softmax(x, axis=axis)
def _gelu(x):
    return jax.nn.gelu(x, approximate=True)
def _silu(x):
    return jax.nn.silu(x)
def _sigmoid(x):
    return jax.nn.sigmoid(x)
def _layernorm(x, axis=-1, eps=1e-5):
    m = jnp.mean(x, axis=axis, keepdims=True)
    v = jnp.var(x, axis=axis, keepdims=True)
    return (x - m) / jnp.sqrt(v + eps)
def _scatter_add(tgt, idx, src, axis=0):
    return tgt.at[idx].add(src)
def _segment_sum(src, seg, n):
    return jax.ops.segment_sum(src, seg, n)
class _Rng:
    def __init__(self, key):
        self._k = key
    def _next(self):
        self._k, sub = jax.random.split(self._k)
        return sub
    def normal(self, shape):
        return jax.random.normal(self._next(), shape, dtype=jnp.bfloat16)
    def randint(self, lo, hi, shape):
        return jax.random.randint(self._next(), shape, lo, hi, dtype=jnp.int32)
    def uniform(self, shape, lo=0.0, hi=1.0):
        return jax.random.uniform(self._next(), shape, jnp.bfloat16, lo, hi)
    def permutation(self, n):
        return jax.random.permutation(self._next(), n)


kernel_name = 'interleave_layers__sliding_local_dilated__spectral_gfnet__prompt'

def setup_inputs():
    _rng = _Rng(jax.random.key(int.from_bytes(__import__("os").urandom(4), "little")))
    _w = (lambda a: (lambda t: t.astype(jnp.bfloat16) if jnp.issubdtype(t.dtype, jnp.floating) else t)(jnp.asarray(a)))
    def _A_setup():
        B, S, D = 1, 2048, 1024
        return {
            "x": _w((lambda *s: _rng.normal(s) * 0.05)(B, S, D)),
            "wqkv": _w((lambda *s: _rng.normal(s) * 0.05)(D, 3 * D)),
            "wo": _w((lambda *s: _rng.normal(s) * 0.05)(D, D)),
        }
    _A_in = _A_setup()

    def _B_setup():
        B, S, D = 1, 2048, 1024
        Df = D // 2 + 1
        return {
            "x": _w((lambda *s: _rng.normal(s) * 0.05)(B, S, D)),
            "w_r": _w((lambda *s: _rng.normal(s) * 0.05)(S, Df) * 0.02),
            "w_i": _w((lambda *s: _rng.normal(s) * 0.05)(S, Df) * 0.02),
        }
    _B_in = _B_setup()

    return {
        "A_x": _A_in["x"],
        "A_wqkv": _A_in["wqkv"],
        "A_wo": _A_in["wo"],
        "B_x": _B_in["x"],
        "B_w_r": _B_in["w_r"],
        "B_w_i": _B_in["w_i"],
    }

def reference(A_x, A_wqkv, A_wo, B_x, B_w_r, B_w_i):
    def _A_ref(x, wqkv, wo):
        B, S, D = x.shape
        H = 32; Dh = D // H
        W, dil = 8, 2
        qkv = (lambda x, *d: x.transpose(*d))((x @ wqkv).reshape(B, S, 3, H, Dh), 2, 0, 3, 1, 4)
        q, k, v = qkv[0], qkv[1], qkv[2]
        scale = Dh ** -0.5
        pos = jnp.arange(S)
        off = jnp.arange(W) * dil
        idx = pos[:, None] - off[None, :]
        mask = idx >= 0
        idx_c = jnp.where(mask, idx, 0).reshape(-1)
        kg = k[:, :, idx_c, :].reshape(B, H, S, W, Dh)
        vg = v[:, :, idx_c, :].reshape(B, H, S, W, Dh)
        logits = jnp.einsum("bhsd,bhswd->bhsw", q, kg) * scale
        logits = jnp.where(mask[None, None, :, :], logits, -1e9)
        attn = _softmax(logits, axis=-1)
        o = jnp.einsum("bhsw,bhswd->bhsd", attn, vg)
        return (lambda x, *d: x.transpose(*d))(o, 0, 2, 1, 3).reshape(B, S, D) @ wo

    def _B_ref(x, w_r, w_i):
        B, S, D = x.shape
        X = (lambda x, axes=(-2,-1): jnp.fft.rfft2(x.astype(jnp.float32), axes=axes))(x, axes=(-2, -1))
        W = w_r + 1j * w_i
        X = X * W
        y = (lambda x, s, axes=(-2,-1): jnp.fft.irfft2(x, s=s, axes=axes).astype(jnp.bfloat16))(X, (S, D), axes=(-2, -1))
        return y

    x = A_x
    x = x + _A_ref(_layernorm(x, axis=-1), A_wqkv, A_wo)
    x = x + _B_ref(_layernorm(x, axis=-1), B_w_r, B_w_i)
    x = x + _A_ref(_layernorm(x, axis=-1), A_wqkv, A_wo)
    x = x + _B_ref(_layernorm(x, axis=-1), B_w_r, B_w_i)
    return x
```

```python
import numpy as np
import jax
import jax.numpy as jnp
from jax import lax
import jax.experimental.pallas as pl
import jax.experimental.pallas.tpu as pltpu

S, D, H, DH, WIN = 2048, 1024, 32, 32, 8
R = 256
NC = S // R
HALO = 128
F32, BF16 = jnp.float32, jnp.bfloat16
C8 = float(np.sqrt(0.5))


def _consts():
    d2 = np.arange(128)[:, None].astype(np.float64)
    k2 = np.arange(128)[None, :]
    md = np.zeros((4, 256, 256))
    kcol = np.zeros((4, 128), np.int64)
    for g, k1 in ((0, 0), (1, 4)):
        kd = k1 + 8 * np.arange(64)[None, :]
        th = 2 * np.pi * kd * d2 / D
        md[0, g * 128:(g + 1) * 128, g * 64:(g + 1) * 64] = np.cos(th)
        md[0, g * 128:(g + 1) * 128, 128 + g * 64:128 + (g + 1) * 64] = -np.sin(th)
        kcol[0, g * 64:(g + 1) * 64] = kd[0]
    md[0, :, 0] = 0.0
    for k1, sg in ((1, -1.0), (2, -1.0), (3, 1.0)):
        kd = k1 + 8 * k2
        th = 2 * np.pi * kd * d2 / D
        cj = np.where(k2 < 64, 1.0, -1.0)
        md[k1, :128, :128] = np.cos(th)
        md[k1, 128:, :128] = sg * np.sin(th)
        md[k1, :128, 128:] = -np.sin(th) * cj
        md[k1, 128:, 128:] = sg * np.cos(th) * cj
        kcol[k1] = np.where(k2 < 64, kd, D - kd)[0]
    mdi = md.transpose(0, 2, 1) * (2.0 / D)
    ab = np.zeros((2, 128, 128))
    ab[0, :, 0] = 1.0
    ab[0, :, 1] = (-1.0) ** np.arange(128)
    ab[1] = ab[0].T / D
    perm = np.zeros((512, 512))
    perm[kcol.reshape(-1), np.arange(512)] = 1.0
    i = np.arange(128)
    s2 = (i // 8 + 16 * (i % 8))[None, :]
    kk = np.arange(128)[:, None]
    ms = np.zeros((16, 256, 256))
    for s1 in range(16):
        th = 2 * np.pi * (kk * (s1 + 16 * s2) % S) / S
        mr, mi = np.cos(th), -np.sin(th)
        ms[s1] = np.block([[mr, -mi], [mi, mr]])
    msi = ms.transpose(0, 2, 1) / S
    return tuple(np.asarray(a, np.float32).astype(jnp.bfloat16) for a in (md, mdi, ab, perm, ms, msi))


def _loop(name, *a):
    with jax.named_scope(name):
        lax.fori_loop(*a)


def _dot(a, b):
    return jnp.dot(a, b, preferred_element_type=F32)


def _dot_nt(a, b):
    return lax.dot_general(a, b, (((1,), (1,)), ((), ())), preferred_element_type=F32)


def _ln(x):
    m = jnp.mean(x, axis=-1, keepdims=True)
    xc = x - m
    v = jnp.mean(xc * xc, axis=-1, keepdims=True)
    return xc * lax.rsqrt(v + 1e-5)


def _bf4(a, b, c, d, sg):
    pr, pi, qr, qi = a[0] + c[0], a[1] + c[1], a[0] - c[0], a[1] - c[1]
    rr, ri, tr, ti = b[0] + d[0], b[1] + d[1], b[0] - d[0], b[1] - d[1]
    y1, y3 = (qr + ti, qi - tr), (qr - ti, qi + tr)
    if sg > 0:
        y1, y3 = y3, y1
    return [(pr + rr, pi + ri), y1, (pr - rr, pi - ri), y3]


def _tw(z, e, sg):
    zr, zi = z
    if e == 0:
        return z
    if e == 4:
        return (-zi, zr) if sg > 0 else (zi, -zr)
    c, s = float(np.cos(2 * np.pi * e / 16)), float(sg * np.sin(2 * np.pi * e / 16))
    if e in (2, 6):
        if c * s > 0:
            return (zr - zi) * c, (zr + zi) * c
        return (zr + zi) * c, (zi - zr) * c
    return zr * c - zi * s, zr * s + zi * c


def _fft16(z, sg):
    cols = [_bf4(z[n], z[n + 4], z[n + 8], z[n + 12], sg) for n in range(4)]
    out = [None] * 16
    for ka in range(4):
        y = _bf4(*[_tw(cols[n][ka], n * ka, sg) for n in range(4)], sg)
        for kb in range(4):
            out[ka + 4 * kb] = y[kb]
    return out


def _kernel(x_hbm, wqkv_hbm, wo_hbm, wr_hbm, wi_hbm, md_hbm, mdi_hbm, ab_hbm, pm_hbm, ms_hbm, msi_hbm,
            o_hbm,
            xio, wqkv_v, wo_v, wr_v, wi_v, md, mdi, ab, pm, ms, msi,
            xs, qb, kb, vb, ure, uim, wt, wop, wp, tmp, ob, sems):
    srcs = (x_hbm, wqkv_hbm, wo_hbm, md_hbm, ab_hbm, wr_hbm, wi_hbm, pm_hbm, ms_hbm, msi_hbm, mdi_hbm)
    dsts = (xio, wqkv_v, wo_v, md, ab, wr_v, wi_v, pm, ms, msi, mdi)
    cps = [pltpu.make_async_copy(s, d, sems.at[i]) for i, (s, d) in enumerate(zip(srcs, dsts))]
    for c in cps:
        c.start()

    def rows(c, off=0):
        return pl.ds(pl.multiple_of(c * R + off, 8), R)

    def xget(c):
        return jnp.concatenate([xs[j, rows(c), :] for j in range(8)], axis=1)

    def xset(c, x):
        for j in range(8):
            xs[j, rows(c), :] = x[:, j * 128:(j + 1) * 128]

    cps[0].wait()
    for b in range(8):
        for j in range(8):
            xs[j, pl.ds(b, 256, stride=8), :] = xio[pl.ds(b * 256, 256), j * 128:(j + 1) * 128].astype(F32)
    cps[1].wait()

    def prep_w(kblk, _):
        k0 = pl.multiple_of(kblk * 128, 128)
        for m in range(3):
            tmp[m] = wqkv_v[pl.ds(k0, 128), m * D:(m + 1) * D].astype(F32).T
            for dd in range(DH):
                wt[kblk, m * D + dd * H:m * D + (dd + 1) * H, :] = (
                    tmp[m, pl.ds(dd, H, stride=DH), :].astype(BF16))
    _loop('prep_w', 0, 8, prep_w, None)

    def prep_wo():
        for kblk in range(8):
            tmp[kblk % 3] = wo_v[:, kblk * 128:(kblk + 1) * 128].astype(F32)
            for dd in range(DH):
                wop[dd * H:(dd + 1) * H, kblk * 128:(kblk + 1) * 128] = (
                    tmp[kblk % 3, pl.ds(dd, H, stride=DH), :].astype(BF16))

    def prep_filter(c, _):
        rs = rows(c)
        lane = lax.broadcasted_iota(jnp.int32, (R, 128), 1)
        for i, w in enumerate((wr_v, wi_v)):
            wp[i, rs, :512] = _dot(w[rs, :512], pm[...]).astype(BF16)
            w0 = w[rs, 0:1].astype(F32)
            w1 = w[rs, 512:513].astype(F32)
            wp[i, rs, 512:] = jnp.where(lane == 0, w0, jnp.where(lane == 1, w1, 0.0)).astype(BF16)

    def qkv(c, x):
        xn = _ln(x).astype(BF16)
        for m, (buf, off) in enumerate(((qb, 0), (kb, HALO), (vb, HALO))):
            wm = jnp.concatenate([wt[j, m * D:(m + 1) * D, :] for j in range(8)], axis=1)
            buf[rows(c, off), :] = _dot_nt(xn, wm)

    def halo():
        sub = lax.broadcasted_iota(jnp.int32, (8, D), 0)
        for buf in (kb, vb):
            for t in range(16):
                z = pltpu.roll(buf[S + 8 * t:S + 8 * t + 8, :], 1, 0)
                buf[8 * t:8 * t + 8, :] = jnp.where(sub == 0, 0.0, z)

    scale = DH ** -0.5

    def attn16(r0):
        sub = lax.broadcasted_iota(jnp.int32, (16, 128), 0)
        key = jnp.where((sub & 7) == 0, r0 + sub, S)
        ls = []
        for w in range(WIN):
            ks = pl.ds(pl.multiple_of(r0 + HALO - 16 * w, 8), 16)
            acc = None
            for j in range(8):
                cs = slice(j * 128, (j + 1) * 128)
                p = qb[pl.ds(r0, 16), cs] * kb[ks, cs]
                acc = p if acc is None else acc + p
            acc = acc + pltpu.roll(acc, 64, 1)
            acc = acc + pltpu.roll(acc, 32, 1)
            if w:
                acc = jnp.where(key < 16 * w, -1e9 / scale, acc)
            ls.append(acc)
        mx = ls[0]
        for l in ls[1:]:
            mx = jnp.maximum(mx, l)
        ps = [jnp.exp2((l - mx) * (scale * float(np.log2(np.e)))) for l in ls]
        den = ps[0]
        for p in ps[1:]:
            den = den + p
        inv = 1.0 / den
        ps = [p * inv for p in ps]
        outs = []
        for j in range(8):
            cs = slice(j * 128, (j + 1) * 128)
            acc = None
            for w in range(WIN):
                p = ps[w] * vb[pl.ds(pl.multiple_of(r0 + HALO - 16 * w, 8), 16), cs]
                acc = p if acc is None else acc + p
            outs.append(acc.astype(BF16))
        return outs

    def attn_chunk(c):
        for i in range(R // 16):
            outs = attn16(pl.multiple_of(c * R + 16 * i, 16))
            for j in range(8):
                ob[16 * i:16 * i + 16, j * 128:(j + 1) * 128] = outs[j]

    def dfwd(c, x):
        xn = _ln(x)
        y = [xn[:, j * 128:(j + 1) * 128] for j in range(8)]
        a = [y[j] + y[j + 4] for j in range(4)]
        b = [y[j] - y[j + 4] for j in range(4)]
        e, f = a[0] + a[2], a[1] + a[3]
        u, v = (b[1] - b[3]) * C8, (b[1] + b[3]) * C8
        ys = [(e + f, e - f), (b[0] + u, b[2] + v), (a[0] - a[2], a[1] - a[3]), (b[0] - u, b[2] - v)]
        rs = rows(c)
        for k1 in range(4):
            lhs = jnp.concatenate([ys[k1][0].astype(BF16), ys[k1][1].astype(BF16)], axis=1)
            z = _dot(lhs, md[k1])
            ure[rs, k1 * 128:(k1 + 1) * 128] = z[:, :128]
            uim[rs, k1 * 128:(k1 + 1) * 128] = z[:, 128:]
        ure[rs, 512:640] = _dot(ys[0][0].astype(BF16), ab[0])

    def gather(buf, s1, cs):
        return jnp.concatenate([buf[pl.ds(pl.multiple_of(128 * j + 8 * s1, 8), 8), cs] for j in range(16)], axis=0)

    def sstage():
        def fwd(s1, _):
            rhs = jnp.concatenate([gather(ure, s1, slice(0, 512)), gather(uim, s1, slice(0, 512))], axis=0)
            z = _dot(ms[s1], rhs.astype(BF16))
            rs = pl.ds(pl.multiple_of(s1 * 128, 128), 128)
            kb[rs, :512] = z[:128]
            vb[rs, :512] = z[128:]
            z = _dot(ms[s1, :, :128], gather(ure, s1, slice(512, 640)).astype(BF16))
            kb[rs, 512:640] = z[:128]
            vb[rs, 512:640] = z[128:]
        _loop('fwd', 0, 16, fwd, None)

        def mid(g, _):
            for cb in range(5):
                cs = slice(cb * 128, (cb + 1) * 128)
                rr = [pl.ds(pl.multiple_of(128 * n + 16 * g, 16), 16) for n in range(16)]
                z = _fft16([(kb[r, cs], vb[r, cs]) for r in rr], -1)
                y = []
                for n in range(16):
                    wr, wi = wp[0, rr[n], cs].astype(F32), wp[1, rr[n], cs].astype(F32)
                    y.append((z[n][0] * wr - z[n][1] * wi, z[n][0] * wi + z[n][1] * wr))
                z = _fft16(y, 1)
                for n in range(16):
                    kb[rr[n], cs] = z[n][0]
                    vb[rr[n], cs] = z[n][1]
        _loop('mid', 0, 8, mid, None)

        def inv(s1, _):
            rs = pl.ds(pl.multiple_of(s1 * 128, 128), 128)
            rhs = jnp.concatenate([kb[rs, :640], vb[rs, :640]], axis=0).astype(BF16)
            z = _dot(msi[s1], rhs[:, :512])
            ze = _dot(msi[s1, :128, :], rhs[:, 512:])
            for j in range(16):
                ro = pl.ds(pl.multiple_of(128 * j + 8 * s1, 8), 8)
                ure[ro, :512] = z[8 * j:8 * j + 8]
                uim[ro, :512] = z[128 + 8 * j:128 + 8 * j + 8]
                ure[ro, 512:640] = ze[8 * j:8 * j + 8]
        _loop('inv', 0, 16, inv, None)

    def dinv(c):
        rs = rows(c)
        z = []
        for k1 in range(4):
            cs = slice(k1 * 128, (k1 + 1) * 128)
            lhs = jnp.concatenate([ure[rs, cs].astype(BF16), uim[rs, cs].astype(BF16)], axis=1)
            o = _dot(lhs, mdi[k1])
            z.append((o[:, :128], o[:, 128:]))
        y0 = z[0][0] + _dot(ure[rs, 512:640].astype(BF16), ab[1])
        e, f = y0 + z[0][1], y0 - z[0][1]
        a = [e + z[2][0], f + z[2][1], e - z[2][0], f - z[2][1]]
        u, v = z[1][0] - z[3][0], z[1][1] - z[3][1]
        b = [z[1][0] + z[3][0], (u + v) * C8, z[1][1] + z[3][1], (v - u) * C8]
        y = jnp.concatenate([a[j] + b[j] for j in range(4)] + [a[j] - b[j] for j in range(4)], axis=1)
        return xget(c) + y

    def first(c, _):
        qkv(c, xget(c))
    _loop('first', 0, NC, first, None)
    cps[2].wait()
    prep_wo()
    cps[3].wait()
    cps[4].wait()

    def mix(c, _):
        attn_chunk(c)
        x = xget(c) + _dot(ob[...], wop[...])
        xset(c, x)
        dfwd(c, x)

    for layer in range(2):
        halo()
        _loop('mix', 0, NC, mix, None)
        if layer == 0:
            for cp in cps[5:]:
                cp.wait()
            _loop('prep_filter', 0, NC, prep_filter, None)
        sstage()
        if layer == 0:
            def nxt(c, _):
                x = dinv(c)
                xset(c, x)
                qkv(c, x)
            _loop('nxt', 0, NC, nxt, None)
        else:
            def last(c, _):
                xset(c, dinv(c))
            _loop('last', 0, NC, last, None)
    for b in range(8):
        for j in range(8):
            xio[pl.ds(b * 256, 256), j * 128:(j + 1) * 128] = xs[j, pl.ds(b, 256, stride=8), :].astype(BF16)
    out = pltpu.make_async_copy(xio, o_hbm, sems.at[0])
    out.start()
    out.wait()


@jax.jit
def pallas_interleave_layers__sliding_local_dilated__spectral_gfnet__prompt_kernel(
        A_x, A_wqkv, A_wo, B_x, B_w_r, B_w_i):
    del B_x
    consts = _consts()
    vm = pltpu.VMEM
    scratch = [
        vm((S, D), BF16), vm((D, 3 * D), BF16), vm((D, D), BF16), vm((S, 513), BF16), vm((S, 513), BF16),
        vm((4, 256, 256), BF16), vm((4, 256, 256), BF16), vm((2, 128, 128), BF16), vm((512, 512), BF16),
        vm((16, 256, 256), BF16), vm((16, 256, 256), BF16),
        vm((8, S, 128), F32), vm((S, D), F32), vm((S + HALO, D), F32), vm((S + HALO, D), F32),
        vm((S, 640), F32), vm((S, 512), F32),
        vm((8, 3 * D, 128), BF16), vm((D, D), BF16), vm((2, S, 640), BF16), vm((3, D, 128), F32),
        vm((R, D), BF16), pltpu.SemaphoreType.DMA((11,)),
    ]
    out = pl.pallas_call(
        _kernel,
        in_specs=[pl.BlockSpec(memory_space=pl.ANY)] * 11,
        out_specs=pl.BlockSpec(memory_space=pl.ANY),
        out_shape=jax.ShapeDtypeStruct((S, D), BF16),
        scratch_shapes=scratch,
        compiler_params=pltpu.CompilerParams(vmem_limit_bytes=120 * 1024 * 1024),
    )(A_x.reshape(S, D), A_wqkv, A_wo, B_w_r, B_w_i, *consts)
    return out.reshape(1, S, D)
```

```python
import numpy as np
import jax
import jax.numpy as jnp
from jax import lax
import jax.experimental.pallas as pl
import jax.experimental.pallas.tpu as pltpu

S, D, H, DH, WIN = 2048, 1024, 32, 32, 8
R = 256
NC = S // R
NW = 256
HALO = 128
F32, BF16 = jnp.float32, jnp.bfloat16
C8 = float(np.sqrt(0.5))


def _consts():
    d2 = np.arange(128)[:, None].astype(np.float64)
    k2 = np.concatenate([np.arange(64), 127 - np.arange(64)])[None, :]
    md = np.zeros((4, 256, 256))
    kcol = np.zeros((4, 128), np.int64)
    for g, k1 in ((0, 0), (1, 4)):
        kd = k1 + 8 * np.arange(64)[None, :]
        th = 2 * np.pi * kd * d2 / D
        md[0, g * 128:(g + 1) * 128, g * 64:(g + 1) * 64] = np.cos(th)
        md[0, g * 128:(g + 1) * 128, 128 + g * 64:128 + (g + 1) * 64] = -np.sin(th)
        kcol[0, g * 64:(g + 1) * 64] = kd[0]
    md[0, :, 0] = 0.0
    for k1, sg in ((1, -1.0), (2, -1.0), (3, 1.0)):
        kd = k1 + 8 * k2
        th = 2 * np.pi * kd * d2 / D
        cj = np.where(k2 < 64, 1.0, -1.0)
        md[k1, :128, :128] = np.cos(th)
        md[k1, 128:, :128] = sg * np.sin(th)
        md[k1, :128, 128:] = -np.sin(th) * cj
        md[k1, 128:, 128:] = sg * np.cos(th) * cj
        kcol[k1] = np.where(k2 < 64, kd, D - kd)[0]
    mdi = md.transpose(0, 2, 1) * (2.0 / D)
    ab = np.zeros((2, 128, 128))
    ab[0, :, 0] = 1.0
    ab[0, :, 1] = (-1.0) ** np.arange(128)
    ab[1] = ab[0].T / D
    i = np.arange(128)
    s2 = (i // 8 + 16 * (i % 8))[None, :]
    kk = np.arange(128)[:, None]
    ms = np.zeros((16, 256, 256))
    for s1 in range(16):
        th = 2 * np.pi * (kk * (s1 + 16 * s2) % S) / S
        mr, mi = np.cos(th), -np.sin(th)
        ms[s1] = np.block([[mr, -mi], [mi, mr]])
    msi = ms.transpose(0, 2, 1) / S
    return tuple(np.asarray(a, np.float32).astype(jnp.bfloat16) for a in (md, mdi, ab, ms, msi))


def _loop(name, *a):
    with jax.named_scope(name):
        lax.fori_loop(*a)


def _weave(*gens):
    order = sorted(((i + 0.5) / n, k) for k, (_, n) in enumerate(gens) for i in range(n))
    for _, k in order:
        next(gens[k][0], None)
    for g, _ in gens:
        for _ in g:
            pass


def _dot(a, b):
    return jnp.dot(a, b, preferred_element_type=F32)


def _dot_nt(a, b):
    return lax.dot_general(a, b, (((1,), (1,)), ((), ())), preferred_element_type=F32)


def _ln(x):
    m = jnp.mean(x, axis=-1, keepdims=True)
    xc = x - m
    v = jnp.mean(xc * xc, axis=-1, keepdims=True)
    return xc * lax.rsqrt(v + 1e-5)


def _bf4(a, b, c, d, sg):
    pr, pi, qr, qi = a[0] + c[0], a[1] + c[1], a[0] - c[0], a[1] - c[1]
    rr, ri, tr, ti = b[0] + d[0], b[1] + d[1], b[0] - d[0], b[1] - d[1]
    y1, y3 = (qr + ti, qi - tr), (qr - ti, qi + tr)
    if sg > 0:
        y1, y3 = y3, y1
    return [(pr + rr, pi + ri), y1, (pr - rr, pi - ri), y3]


def _tw(z, e, sg):
    zr, zi = z
    if e == 0:
        return z
    if e == 4:
        return (-zi, zr) if sg > 0 else (zi, -zr)
    c, s = float(np.cos(2 * np.pi * e / 16)), float(sg * np.sin(2 * np.pi * e / 16))
    if e in (2, 6):
        if c * s > 0:
            return (zr - zi) * c, (zr + zi) * c
        return (zr + zi) * c, (zi - zr) * c
    return zr * c - zi * s, zr * s + zi * c


def _fft16(z, sg):
    cols = [_bf4(z[n], z[n + 4], z[n + 8], z[n + 12], sg) for n in range(4)]
    out = [None] * 16
    for ka in range(4):
        y = _bf4(*[_tw(cols[n][ka], n * ka, sg) for n in range(4)], sg)
        for kb in range(4):
            out[ka + 4 * kb] = y[kb]
    return out


def _kernel(x_hbm, wqkv_hbm, wo_hbm, wr_hbm, wi_hbm, md_hbm, mdi_hbm, ab_hbm, ms_hbm, msi_hbm,
            o_hbm,
            xio, wqkv_v, wo_v, wr_v, wi_v, md, mdi, ab, ms, msi,
            xs, qb, kb, vb, ub, wtmp, wt, wop, wp, tmp, ob, sems):
    srcs = (x_hbm, wqkv_hbm, wo_hbm, md_hbm, ab_hbm, wr_hbm, wi_hbm, ms_hbm, msi_hbm, mdi_hbm)
    dsts = (xio, wqkv_v, wo_v, md, ab, wr_v, wi_v, ms, msi, mdi)
    cps = [pltpu.make_async_copy(s, d, sems.at[i]) for i, (s, d) in enumerate(zip(srcs, dsts))]
    cps[0].start()
    cps[1].start()

    def rows(c, off=0):
        return pl.ds(pl.multiple_of(c * R + off, 8), R)

    def xget(c):
        return jnp.concatenate([xs[j, rows(c), :] for j in range(8)], axis=1)

    def xset(c, x):
        for j in range(8):
            xs[j, rows(c), :] = x[:, j * 128:(j + 1) * 128]

    cps[0].wait()
    for b in range(8):
        for j in range(8):
            xs[j, pl.ds(b, 256, stride=8), :] = xio[pl.ds(b * 256, 256), j * 128:(j + 1) * 128].astype(F32)
    cps[1].wait()
    for c in cps[2:]:
        c.start()

    def prep_w(kblk, _):
        k0 = pl.multiple_of(kblk * 128, 128)
        for m in range(3):
            tmp[m] = wqkv_v[pl.ds(k0, 128), m * D:(m + 1) * D].astype(F32).T
            for dd in range(DH):
                wt[kblk, m * D + dd * H:m * D + (dd + 1) * H, :] = (
                    tmp[m, pl.ds(dd, H, stride=DH), :].astype(BF16))
    _loop('prep_w', 0, 8, prep_w, None)

    def prep_wo():
        for kblk in range(8):
            tmp[kblk % 3] = wo_v[:, kblk * 128:(kblk + 1) * 128].astype(F32)
            for dd in range(DH):
                wop[dd * H:(dd + 1) * H, kblk * 128:(kblk + 1) * 128] = (
                    tmp[kblk % 3, pl.ds(dd, H, stride=DH), :].astype(BF16))

    def prep_filter(c):
        sub = lax.broadcasted_iota(jnp.int32, (128, 128), 0)
        for i, w in enumerate((wr_v, wi_v)):
            for h in range(2):
                k0 = pl.multiple_of(c * R + h * 128, 128)
                tw = wtmp.at[2 * i + h]
                tw[...] = w[:512, pl.ds(k0, 128)].astype(F32)
                for k1, (lo, hi) in enumerate(((0, 4), (1, 7), (2, 6), (3, 5))):
                    z = jnp.concatenate([tw[pl.ds(lo, 64, stride=8), :], tw[pl.ds(hi, 64, stride=8), :]], axis=0)
                    wp[i, pl.ds(k0, 128), k1 * 128:(k1 + 1) * 128] = z.T.astype(BF16)
                w1 = w[512:513, pl.ds(k0, 128)].astype(F32)
                z = jnp.where(sub == 0, tw[0:1, :], jnp.where(sub == 1, w1, 0.0))
                wp[i, pl.ds(k0, 128), 512:] = z.T.astype(BF16)
                yield

    def qkv(c, x):
        xn = _ln(x).astype(BF16)
        for m, (buf, off) in enumerate(((qb, 0), (kb, HALO), (vb, HALO))):
            for n in range(0, D, NW):
                wm = jnp.concatenate([wt[j, m * D + n:m * D + n + NW, :] for j in range(8)], axis=1)
                buf[rows(c, off), n:n + NW] = _dot_nt(xn, wm)
                yield

    def halo():
        sub = lax.broadcasted_iota(jnp.int32, (8, D), 0)
        for buf in (kb, vb):
            for t in range(16):
                z = pltpu.roll(buf[S + 8 * t:S + 8 * t + 8, :], 1, 0)
                buf[8 * t:8 * t + 8, :] = jnp.where(sub == 0, 0.0, z)

    scale = DH ** -0.5

    def attn16(r0):
        sub = lax.broadcasted_iota(jnp.int32, (16, 128), 0)
        key = jnp.where((sub & 7) == 0, r0 + sub, S)
        ls = []
        for w in range(WIN):
            ks = pl.ds(pl.multiple_of(r0 + HALO - 16 * w, 8), 16)
            acc = None
            for j in range(8):
                cs = slice(j * 128, (j + 1) * 128)
                p = qb[pl.ds(r0, 16), cs] * kb[ks, cs]
                acc = p if acc is None else acc + p
            acc = acc + pltpu.roll(acc, 64, 1)
            acc = acc + pltpu.roll(acc, 32, 1)
            if w:
                acc = jnp.where(key < 16 * w, -1e9 / scale, acc)
            ls.append(acc)
        mx = ls[0]
        for l in ls[1:]:
            mx = jnp.maximum(mx, l)
        ps = [jnp.exp2((l - mx) * (scale * float(np.log2(np.e)))) for l in ls]
        den = ps[0]
        for p in ps[1:]:
            den = den + p
        inv = 1.0 / den
        ps = [p * inv for p in ps]
        outs = []
        for j in range(8):
            cs = slice(j * 128, (j + 1) * 128)
            acc = None
            for w in range(WIN):
                p = ps[w] * vb[pl.ds(pl.multiple_of(r0 + HALO - 16 * w, 8), 16), cs]
                acc = p if acc is None else acc + p
            outs.append(acc.astype(BF16))
        return outs

    def attn_chunk(c):
        for i in range(R // 16):
            outs = attn16(pl.multiple_of(c * R + 16 * i, 16))
            for j in range(8):
                ob[pl.ds(pl.multiple_of(c * R + 16 * i, 16), 16), j * 128:(j + 1) * 128] = outs[j]
            yield

    def dfwd(c, x):
        xn = _ln(x)
        y = [xn[:, j * 128:(j + 1) * 128] for j in range(8)]
        a = [y[j] + y[j + 4] for j in range(4)]
        b = [y[j] - y[j + 4] for j in range(4)]
        e, f = a[0] + a[2], a[1] + a[3]
        u, v = (b[1] - b[3]) * C8, (b[1] + b[3]) * C8
        ys = [(e + f, e - f), (b[0] + u, b[2] + v), (a[0] - a[2], a[1] - a[3]), (b[0] - u, b[2] - v)]
        ro = pl.ds(pl.multiple_of(16 * c, 16), 16)
        ri = pl.ds(pl.multiple_of(128 + 16 * c, 16), 16)

        def regroup(z):
            return jnp.concatenate([z[128 * jj + 8 * s1:128 * jj + 8 * s1 + 8]
                                    for s1 in range(16) for jj in range(2)], axis=0).astype(BF16)
        for k1 in range(4):
            lhs = jnp.concatenate([regroup(ys[k1][0]), regroup(ys[k1][1])], axis=1)
            z = _dot(lhs, md[k1]).astype(BF16)
            for s1 in range(16):
                ub[s1, ro, k1 * 128:(k1 + 1) * 128] = z[16 * s1:16 * s1 + 16, :128]
                ub[s1, ri, k1 * 128:(k1 + 1) * 128] = z[16 * s1:16 * s1 + 16, 128:]
            if k1 == 0:
                z = _dot(lhs[:, :128], ab[0]).astype(BF16)
                for s1 in range(16):
                    ub[s1, ro, 512:] = z[16 * s1:16 * s1 + 16]
            yield

    def sstage():
        def fwd(s1, _):
            z = _dot(ms[s1], ub[s1, :, :512])
            rs = pl.ds(pl.multiple_of(s1 * 128, 128), 128)
            kb[rs, :512] = z[:128]
            vb[rs, :512] = z[128:]
            z = _dot(ms[s1, :, :128], ub[s1, :128, 512:])
            kb[rs, 512:640] = z[:128]
            vb[rs, 512:640] = z[128:]
        _loop('fwd', 0, 16, fwd, None)

        def mid(g, _):
            for cb in range(5):
                cs = slice(cb * 128, (cb + 1) * 128)
                rr = [pl.ds(pl.multiple_of(128 * n + 16 * g, 16), 16) for n in range(16)]
                z = _fft16([(kb[r, cs], vb[r, cs]) for r in rr], -1)
                y = []
                for n in range(16):
                    wr, wi = wp[0, rr[n], cs].astype(F32), wp[1, rr[n], cs].astype(F32)
                    y.append((z[n][0] * wr - z[n][1] * wi, z[n][0] * wi + z[n][1] * wr))
                z = _fft16(y, 1)
                for n in range(16):
                    ub[n, pl.ds(pl.multiple_of(16 * g, 16), 16), cs] = z[n][0].astype(BF16)
                    ub[n, pl.ds(pl.multiple_of(128 + 16 * g, 16), 16), cs] = z[n][1].astype(BF16)
        _loop('mid', 0, 8, mid, None)

        def inv(s1, _):
            z = _dot(msi[s1], ub[s1, :, :512])
            ze = _dot(msi[s1, :128, :], ub[s1, :, 512:])
            ub[s1, :, :512] = z.astype(BF16)
            ub[s1, :128, 512:] = ze.astype(BF16)
        _loop('inv', 0, 16, inv, None)

    def dinv(c):
        ro = pl.ds(pl.multiple_of(16 * c, 16), 16)
        ri = pl.ds(pl.multiple_of(128 + 16 * c, 16), 16)

        def grab(r, cs):
            return jnp.concatenate([ub[s1, r, cs] for s1 in range(16)], axis=0)
        z = []
        for k1 in range(4):
            cs = slice(k1 * 128, (k1 + 1) * 128)
            o = _dot(jnp.concatenate([grab(ro, cs), grab(ri, cs)], axis=1), mdi[k1])
            z.append((o[:, :128], o[:, 128:]))
        y0 = z[0][0] + _dot(grab(ro, slice(512, 640)), ab[1])
        e, f = y0 + z[0][1], y0 - z[0][1]
        a = [e + z[2][0], f + z[2][1], e - z[2][0], f - z[2][1]]
        u, v = z[1][0] - z[3][0], z[1][1] - z[3][1]
        b = [z[1][0] + z[3][0], (u + v) * C8, z[1][1] + z[3][1], (v - u) * C8]
        y = jnp.concatenate([a[j] + b[j] for j in range(4)] + [a[j] - b[j] for j in range(4)], axis=1)
        y = jnp.concatenate([y[16 * s1 + 8 * jj:16 * s1 + 8 * jj + 8]
                             for jj in range(2) for s1 in range(16)], axis=0)
        return xget(c) + y

    def project(c, layer):
        if layer == 0:
            x = xget(c)
        else:
            x = dinv(c)
            xset(c, x)
        yield from qkv(c, x)

    def mix(c):
        o, xj = ob[rows(c), :], []
        for n in range(0, D, NW):
            xj.append(_dot(o, wop[:, n:n + NW]))
            yield
        x = xget(c) + jnp.concatenate(xj, axis=1)
        xset(c, x)
        yield
        yield from dfwd(c, x)

    def out_copy(c, b):
        return pltpu.make_async_copy(xio.at[pl.ds(b * 256 + c * 32, 32)],
                                     o_hbm.at[pl.ds(b * 256 + c * 32, 32)], sems.at[0])

    for layer in range(2):
        def head(i, _):
            _weave((project((i + NC - 1) % NC, layer), 1))
        _loop('head', 0, 2, head, None)
        halo()

        def body(i, _):
            _weave((project(i + 1, layer), 3 * D // NW), (attn_chunk(i), 16))
        _loop('body', 0, NC - 2, body, None)
        if layer == 0:
            cps[2].wait()
            prep_wo()
            for cp in cps[3:7]:
                cp.wait()

        def extra(i):
            return [(prep_filter(i), 4)] if layer == 0 else []

        def mix_a(i, _):
            _weave((mix(i), D // NW + 5), (attn_chunk(i + NC - 2), 16), *extra(i))
        _loop('mix_a', 0, 2, mix_a, None)
        _loop('mix_b', 2, NC, lambda i, _: _weave((mix(i), D // NW + 5), *extra(i)), None)
        if layer == 0:
            for cp in cps[7:]:
                cp.wait()
        sstage()

    def last(c, _):
        xset(c, dinv(c))
        for b in range(8):
            for j in range(8):
                xio[pl.ds(pl.multiple_of(b * 256 + c * 32, 32), 32), j * 128:(j + 1) * 128] = (
                    xs[j, pl.ds(c * R + b, 32, stride=8), :].astype(BF16))
            out_copy(c, b).start()
    _loop('last', 0, NC, last, None)
    pltpu.make_async_copy(xio, o_hbm, sems.at[0]).wait()


@jax.jit
def pallas_interleave_layers__sliding_local_dilated__spectral_gfnet__prompt_kernel(
        A_x, A_wqkv, A_wo, B_x, B_w_r, B_w_i):
    del B_x
    consts = _consts()
    vm = pltpu.VMEM
    scratch = [
        vm((S, D), BF16), vm((D, 3 * D), BF16), vm((D, D), BF16), vm((513, S), BF16), vm((513, S), BF16),
        vm((4, 256, 256), BF16), vm((4, 256, 256), BF16), vm((2, 128, 128), BF16),
        vm((16, 256, 256), BF16), vm((16, 256, 256), BF16),
        vm((8, S, 128), F32), vm((S, D), F32), vm((S + HALO, D), F32), vm((S + HALO, D), F32),
        vm((16, 256, 640), BF16), vm((4, 512, 128), F32),
        vm((8, 3 * D, 128), BF16), vm((D, D), BF16), vm((2, S, 640), BF16), vm((3, D, 128), F32),
        vm((S, D), BF16), pltpu.SemaphoreType.DMA((10,)),
    ]
    out = pl.pallas_call(
        _kernel,
        in_specs=[pl.BlockSpec(memory_space=pl.ANY)] * 10,
        out_specs=pl.BlockSpec(memory_space=pl.ANY),
        out_shape=jax.ShapeDtypeStruct((S, D), BF16),
        scratch_shapes=scratch,
        compiler_params=pltpu.CompilerParams(vmem_limit_bytes=120 * 1024 * 1024),
    )(A_x.reshape(S, D), A_wqkv, A_wo, B_w_r.T, B_w_i.T, *consts)
    return out.reshape(1, S, D)
```

```python
import numpy as np
import jax
import jax.numpy as jnp
from jax import lax
import jax.experimental.pallas as pl
import jax.experimental.pallas.tpu as pltpu

S, D, H, DH, WIN = 2048, 1024, 32, 32, 8
R = 256
NC = S // R
NW = 256
HALO = 128
F32, BF16 = jnp.float32, jnp.bfloat16
C8 = float(np.sqrt(0.5))


def _consts():
    d2 = np.arange(128)[:, None].astype(np.float64)
    k2 = np.concatenate([np.arange(64), 127 - np.arange(64)])[None, :]
    md = np.zeros((4, 256, 256))
    kcol = np.zeros((4, 128), np.int64)
    for g, k1 in ((0, 0), (1, 4)):
        kd = k1 + 8 * np.arange(64)[None, :]
        th = 2 * np.pi * kd * d2 / D
        md[0, g * 128:(g + 1) * 128, g * 64:(g + 1) * 64] = np.cos(th)
        md[0, g * 128:(g + 1) * 128, 128 + g * 64:128 + (g + 1) * 64] = -np.sin(th)
        kcol[0, g * 64:(g + 1) * 64] = kd[0]
    md[0, :, 0] = 0.0
    for k1, sg in ((1, -1.0), (2, -1.0), (3, 1.0)):
        kd = k1 + 8 * k2
        th = 2 * np.pi * kd * d2 / D
        cj = np.where(k2 < 64, 1.0, -1.0)
        md[k1, :128, :128] = np.cos(th)
        md[k1, 128:, :128] = sg * np.sin(th)
        md[k1, :128, 128:] = -np.sin(th) * cj
        md[k1, 128:, 128:] = sg * np.cos(th) * cj
        kcol[k1] = np.where(k2 < 64, kd, D - kd)[0]
    mdi = md.transpose(0, 2, 1) * (2.0 / D)
    ab = np.zeros((2, 128, 128))
    ab[0, :, 0] = 1.0
    ab[0, :, 1] = (-1.0) ** np.arange(128)
    ab[1] = ab[0].T / D
    i = np.arange(128)
    s2 = (i // 8 + 16 * (i % 8))[None, :]
    kk = np.arange(128)[:, None]
    ms = np.zeros((16, 256, 256))
    for s1 in range(16):
        th = 2 * np.pi * (kk * (s1 + 16 * s2) % S) / S
        mr, mi = np.cos(th), -np.sin(th)
        ms[s1] = np.block([[mr, -mi], [mi, mr]])
    msi = ms.transpose(0, 2, 1) / S
    return tuple(np.asarray(a, np.float32).astype(jnp.bfloat16) for a in (md, mdi, ab, ms, msi))


def _loop(name, *a):
    with jax.named_scope(name):
        lax.fori_loop(*a, unroll=4 if name[0] in 'spl' else 1)


def _weave(*gens):
    order = sorted(((i + 0.5) / n, k) for k, (_, n) in enumerate(gens) for i in range(n))
    for _, k in order:
        next(gens[k][0], None)
    for g, _ in gens:
        for _ in g:
            pass


def _dot(a, b):
    return jnp.dot(a, b, preferred_element_type=F32)


def _dot_nt(a, b):
    return lax.dot_general(a, b, (((1,), (1,)), ((), ())), preferred_element_type=F32)


def _ln(x):
    m = jnp.mean(x, axis=-1, keepdims=True)
    xc = x - m
    v = jnp.mean(xc * xc, axis=-1, keepdims=True)
    return xc * lax.rsqrt(v + 1e-5)


def _bf4(a, b, c, d, sg):
    pr, pi, qr, qi = a[0] + c[0], a[1] + c[1], a[0] - c[0], a[1] - c[1]
    rr, ri, tr, ti = b[0] + d[0], b[1] + d[1], b[0] - d[0], b[1] - d[1]
    y1, y3 = (qr + ti, qi - tr), (qr - ti, qi + tr)
    if sg > 0:
        y1, y3 = y3, y1
    return [(pr + rr, pi + ri), y1, (pr - rr, pi - ri), y3]


def _tw(z, e, sg):
    zr, zi = z
    if e == 0:
        return z
    if e == 4:
        return (-zi, zr) if sg > 0 else (zi, -zr)
    c, s = float(np.cos(2 * np.pi * e / 16)), float(sg * np.sin(2 * np.pi * e / 16))
    if e in (2, 6):
        if c * s > 0:
            return (zr - zi) * c, (zr + zi) * c
        return (zr + zi) * c, (zi - zr) * c
    return zr * c - zi * s, zr * s + zi * c


def _fft16(z, sg):
    cols = [_bf4(z[n], z[n + 4], z[n + 8], z[n + 12], sg) for n in range(4)]
    out = [None] * 16
    for ka in range(4):
        y = _bf4(*[_tw(cols[n][ka], n * ka, sg) for n in range(4)], sg)
        for kb in range(4):
            out[ka + 4 * kb] = y[kb]
    return out


def _kernel(x_hbm, wqkv_hbm, wo_hbm, wr_hbm, wi_hbm, md_hbm, mdi_hbm, ab_hbm, ms_hbm, msi_hbm,
            o_hbm,
            xio, wqkv_v, wo_v, wr_v, wi_v, md, mdi, ab, ms, msi,
            xs, qb, kb, vb, ub, wtmp, wt, wop, wp, tmp, ob, sems, wsems):
    srcs = (x_hbm, wqkv_hbm, wo_hbm, md_hbm, ab_hbm, wr_hbm, wi_hbm, ms_hbm, msi_hbm, mdi_hbm)
    dsts = (xio, wqkv_v, wo_v, md, ab, wr_v, wi_v, ms, msi, mdi)
    cps = [None if i == 1 else pltpu.make_async_copy(s, d, sems.at[i])
           for i, (s, d) in enumerate(zip(srcs, dsts))]

    def w_copy(k):
        ks = pl.ds(pl.multiple_of(k * 128, 128), 128)
        return pltpu.make_async_copy(wqkv_hbm.at[ks], wqkv_v.at[ks], wsems.at[k])
    for k in range(8):
        w_copy(k).start()
    cps[0].start()

    def rows(c, off=0):
        return pl.ds(pl.multiple_of(c * R + off, 8), R)

    def xget(c):
        return jnp.concatenate([xs[j, rows(c), :] for j in range(8)], axis=1)

    def xset(c, x):
        for j in range(8):
            xs[j, rows(c), :] = x[:, j * 128:(j + 1) * 128]

    def prep_w(kblk, _):
        k0 = pl.multiple_of(kblk * 128, 128)
        w_copy(kblk).wait()
        for m in range(3):
            tmp[m] = wqkv_v[pl.ds(k0, 128), m * D:(m + 1) * D].astype(F32).T
            for dd in range(DH):
                wt[kblk, m * D + dd * H:m * D + (dd + 1) * H, :] = (
                    tmp[m, pl.ds(dd, H, stride=DH), :].astype(BF16))
    _loop('prep_w', 0, 8, prep_w, None)

    cps[0].wait()
    for c in cps[2:]:
        c.start()
    for b in range(8):
        for j in range(8):
            xs[j, pl.ds(b, 256, stride=8), :] = xio[pl.ds(b * 256, 256), j * 128:(j + 1) * 128].astype(F32)

    def prep_wo():
        for kblk in range(8):
            tmp[kblk % 3] = wo_v[:, kblk * 128:(kblk + 1) * 128].astype(F32)
            for dd in range(DH):
                wop[dd * H:(dd + 1) * H, kblk * 128:(kblk + 1) * 128] = (
                    tmp[kblk % 3, pl.ds(dd, H, stride=DH), :].astype(BF16))

    def prep_filter(c):
        sub = lax.broadcasted_iota(jnp.int32, (128, 128), 0)
        for i, w in enumerate((wr_v, wi_v)):
            for h in range(2):
                k0 = pl.multiple_of(c * R + h * 128, 128)
                tw = wtmp.at[2 * i + h]
                tw[...] = w[:512, pl.ds(k0, 128)].astype(F32)
                for k1, (lo, hi) in enumerate(((0, 4), (1, 7), (2, 6), (3, 5))):
                    z = jnp.concatenate([tw[pl.ds(lo, 64, stride=8), :], tw[pl.ds(hi, 64, stride=8), :]], axis=0)
                    wp[i, pl.ds(k0, 128), k1 * 128:(k1 + 1) * 128] = z.T.astype(BF16)
                w1 = w[512:513, pl.ds(k0, 128)].astype(F32)
                z = jnp.where(sub == 0, tw[0:1, :], jnp.where(sub == 1, w1, 0.0))
                wp[i, pl.ds(k0, 128), 512:] = z.T.astype(BF16)
                yield

    def qkv(c, x):
        xn = _ln(x).astype(BF16)
        for m, (buf, off) in enumerate(((qb, 0), (kb, HALO), (vb, HALO))):
            for n in range(0, D, NW):
                wm = jnp.concatenate([wt[j, m * D + n:m * D + n + NW, :] for j in range(8)], axis=1)
                buf[rows(c, off), n:n + NW] = _dot_nt(xn, wm)
                yield

    def halo():
        sub = lax.broadcasted_iota(jnp.int32, (8, D), 0)
        for buf in (kb, vb):
            for t in range(16):
                z = pltpu.roll(buf[S + 8 * t:S + 8 * t + 8, :], 1, 0)
                buf[8 * t:8 * t + 8, :] = jnp.where(sub == 0, 0.0, z)

    scale = DH ** -0.5

    def attn16(r0):
        sub = lax.broadcasted_iota(jnp.int32, (16, 128), 0)
        key = jnp.where((sub & 7) == 0, r0 + sub, S)
        ls = []
        for w in range(WIN):
            ks = pl.ds(pl.multiple_of(r0 + HALO - 16 * w, 8), 16)
            acc = None
            for j in range(8):
                cs = slice(j * 128, (j + 1) * 128)
                p = qb[pl.ds(r0, 16), cs] * kb[ks, cs]
                acc = p if acc is None else acc + p
            acc = acc + pltpu.roll(acc, 64, 1)
            acc = acc + pltpu.roll(acc, 32, 1)
            if w:
                acc = jnp.where(key < 16 * w, -1e9 / scale, acc)
            ls.append(acc)
        mx = ls[0]
        for l in ls[1:]:
            mx = jnp.maximum(mx, l)
        ps = [jnp.exp2((l - mx) * (scale * float(np.log2(np.e)))) for l in ls]
        den = ps[0]
        for p in ps[1:]:
            den = den + p
        inv = 1.0 / den
        ps = [p * inv for p in ps]
        outs = []
        for j in range(8):
            cs = slice(j * 128, (j + 1) * 128)
            acc = None
            for w in range(WIN):
                p = ps[w] * vb[pl.ds(pl.multiple_of(r0 + HALO - 16 * w, 8), 16), cs]
                acc = p if acc is None else acc + p
            outs.append(acc.astype(BF16))
        return outs

    def attn_chunk(r0, n):
        for i in range(n):
            outs = attn16(pl.multiple_of(r0 + 16 * i, 16))
            for j in range(8):
                ob[pl.ds(pl.multiple_of(r0 + 16 * i, 16), 16), j * 128:(j + 1) * 128] = outs[j]
            yield

    def dfwd(c):
        xn = _ln(xget(c))
        y = [xn[:, j * 128:(j + 1) * 128] for j in range(8)]
        a = [y[j] + y[j + 4] for j in range(4)]
        b = [y[j] - y[j + 4] for j in range(4)]
        e, f = a[0] + a[2], a[1] + a[3]
        u, v = (b[1] - b[3]) * C8, (b[1] + b[3]) * C8
        ys = [(e + f, e - f), (b[0] + u, b[2] + v), (a[0] - a[2], a[1] - a[3]), (b[0] - u, b[2] - v)]
        ro = pl.ds(pl.multiple_of(16 * c, 16), 16)
        ri = pl.ds(pl.multiple_of(128 + 16 * c, 16), 16)

        def regroup(z):
            return jnp.concatenate([z[128 * jj + 8 * s1:128 * jj + 8 * s1 + 8]
                                    for s1 in range(16) for jj in range(2)], axis=0).astype(BF16)
        for k1 in range(4):
            lhs = jnp.concatenate([regroup(ys[k1][0]), regroup(ys[k1][1])], axis=1)
            z = _dot(lhs, md[k1]).astype(BF16)
            for s1 in range(16):
                ub[s1, ro, k1 * 128:(k1 + 1) * 128] = z[16 * s1:16 * s1 + 16, :128]
                ub[s1, ri, k1 * 128:(k1 + 1) * 128] = z[16 * s1:16 * s1 + 16, 128:]
            if k1 == 0:
                z = _dot(lhs[:, :128], ab[0]).astype(BF16)
                for s1 in range(16):
                    ub[s1, ro, 512:] = z[16 * s1:16 * s1 + 16]
            yield

    def sstage():
        def fwd(s1, cb):
            cs = slice(cb * 128, (cb + 1) * 128)
            kk = 256 if cb < 4 else 128
            z = _dot(ms[s1, :, :kk], ub[s1, :kk, cs])
            rs = pl.ds(pl.multiple_of(s1 * 128, 128), 128)
            tb = (kb, vb)[cb % 2]
            tb[rs, :128] = z[:128]
            tb[rs, 128:256] = z[128:]

        def mid(g, cb):
            cs = slice(cb * 128, (cb + 1) * 128)
            tb = (kb, vb)[cb % 2]
            rr = [pl.ds(pl.multiple_of(128 * n + 16 * g, 16), 16) for n in range(16)]
            z = _fft16([(tb[r, :128], tb[r, 128:256]) for r in rr], -1)
            yield
            y = []
            for n in range(16):
                wr, wi = wp[0, rr[n], cs].astype(F32), wp[1, rr[n], cs].astype(F32)
                y.append((z[n][0] * wr - z[n][1] * wi, z[n][0] * wi + z[n][1] * wr))
            yield
            z = _fft16(y, 1)
            for n in range(16):
                ob[rr[n], cb % 2 * 256:cb % 2 * 256 + 128] = z[n][0].astype(BF16)
                ob[rr[n], cb % 2 * 256 + 128:cb % 2 * 256 + 256] = z[n][1].astype(BF16)
            yield

        def inv(s1, cb):
            kk = 256 if cb < 4 else 128
            rs = pl.ds(pl.multiple_of(s1 * 128, 128), 128)
            o = cb % 2 * 256
            rhs = jnp.concatenate([ob[rs, o:o + 128], ob[rs, o + 128:o + 256]], axis=0)
            ub[s1, :kk, cb * 128:(cb + 1) * 128] = _dot(msi[s1, :kk, :], rhs).astype(BF16)

        for t in range(7):
            def mats(g):
                for h in range(2):
                    if t >= 2:
                        inv(2 * g + h, t - 2)
                    yield
                    if t < 5:
                        fwd(2 * g + h, t)
                    yield

            def step(g, _):
                _weave((mats(g), 4), *([(mid(g, t - 1), 3)] if 1 <= t < 6 else []))
            _loop('s%d' % t, 0, 8, step, None)

    def dinv(c):
        ro = pl.ds(pl.multiple_of(16 * c, 16), 16)
        ri = pl.ds(pl.multiple_of(128 + 16 * c, 16), 16)

        def grab(r, cs):
            return jnp.concatenate([ub[s1, r, cs] for s1 in range(16)], axis=0)
        z = []
        for k1 in range(4):
            cs = slice(k1 * 128, (k1 + 1) * 128)
            o = _dot(jnp.concatenate([grab(ro, cs), grab(ri, cs)], axis=1), mdi[k1])
            z.append((o[:, :128], o[:, 128:]))
        y0 = z[0][0] + _dot(grab(ro, slice(512, 640)), ab[1])
        e, f = y0 + z[0][1], y0 - z[0][1]
        a = [e + z[2][0], f + z[2][1], e - z[2][0], f - z[2][1]]
        u, v = z[1][0] - z[3][0], z[1][1] - z[3][1]
        b = [z[1][0] + z[3][0], (u + v) * C8, z[1][1] + z[3][1], (v - u) * C8]
        y = jnp.concatenate([a[j] + b[j] for j in range(4)] + [a[j] - b[j] for j in range(4)], axis=1)
        y = jnp.concatenate([y[16 * s1 + 8 * jj:16 * s1 + 8 * jj + 8]
                             for jj in range(2) for s1 in range(16)], axis=0)
        return xget(c) + y

    def project(c, layer):
        if layer == 0:
            x = xget(c)
        else:
            x = dinv(c)
            xset(c, x)
        yield from qkv(c, x)

    def mix(c):
        o, xj = ob[rows(c), :], []
        for n in range(0, D, NW):
            xj.append(_dot(o, wop[:, n:n + NW]))
            yield
        x = xget(c) + jnp.concatenate(xj, axis=1)
        xset(c, x)

    def out_copy(c, b):
        return pltpu.make_async_copy(xio.at[pl.ds(b * 256 + c * 32, 32)],
                                     o_hbm.at[pl.ds(b * 256 + c * 32, 32)], sems.at[0])

    for layer in range(2):
        def head(i, _):
            _weave((project((i + NC - 1) % NC, layer), 1))
        _loop('head', 0, 2, head, None)
        halo()

        def body(i, _):
            _weave((project(i + 1, layer), 3 * D // NW), (attn_chunk(i * R, 16), 16))
        _loop('body', 0, NC - 2, body, None)
        if layer == 0:
            cps[2].wait()
            prep_wo()
            for cp in cps[3:7]:
                cp.wait()

        def extra(i):
            return [(prep_filter(i), 4)] if layer == 0 else []

        _weave((mix(0), 1))

        def mix_a(i, _):
            _weave((dfwd(i), 4), (mix(i + 1), D // NW), (attn_chunk((NC - 2) * R + 128 * i, 8), 8), *extra(i))
        _loop('mix_a', 0, 4, mix_a, None)
        _loop('mix_b', 4, NC - 1, lambda i, _: _weave((dfwd(i), 4), (mix(i + 1), D // NW), *extra(i)), None)
        _weave((dfwd(NC - 1), 4), *extra(NC - 1))
        if layer == 0:
            for cp in cps[7:]:
                cp.wait()
        sstage()

    def last(c, _):
        xset(c, dinv(c))
        for b in range(8):
            for j in range(8):
                xio[pl.ds(pl.multiple_of(b * 256 + c * 32, 32), 32), j * 128:(j + 1) * 128] = (
                    xs[j, pl.ds(c * R + b, 32, stride=8), :].astype(BF16))
            out_copy(c, b).start()
    _loop('last', 0, NC, last, None)
    pltpu.make_async_copy(xio, o_hbm, sems.at[0]).wait()


@jax.jit
def pallas_interleave_layers__sliding_local_dilated__spectral_gfnet__prompt_kernel(
        A_x, A_wqkv, A_wo, B_x, B_w_r, B_w_i):
    del B_x
    consts = _consts()
    vm = pltpu.VMEM
    scratch = [
        vm((S, D), BF16), vm((D, 3 * D), BF16), vm((D, D), BF16), vm((513, S), BF16), vm((513, S), BF16),
        vm((4, 256, 256), BF16), vm((4, 256, 256), BF16), vm((2, 128, 128), BF16),
        vm((16, 256, 256), BF16), vm((16, 256, 256), BF16),
        vm((8, S, 128), F32), vm((S, D), F32), vm((S + HALO, D), F32), vm((S + HALO, D), F32),
        vm((16, 256, 640), BF16), vm((4, 512, 128), F32),
        vm((8, 3 * D, 128), BF16), vm((D, D), BF16), vm((2, S, 640), BF16), vm((3, D, 128), F32),
        vm((S, D), BF16), pltpu.SemaphoreType.DMA((10,)), pltpu.SemaphoreType.DMA((8,)),
    ]
    out = pl.pallas_call(
        _kernel,
        in_specs=[pl.BlockSpec(memory_space=pl.ANY)] * 10,
        out_specs=pl.BlockSpec(memory_space=pl.ANY),
        out_shape=jax.ShapeDtypeStruct((S, D), BF16),
        scratch_shapes=scratch,
        compiler_params=pltpu.CompilerParams(vmem_limit_bytes=120 * 1024 * 1024),
    )(A_x.reshape(S, D), A_wqkv, A_wo, B_w_r.T, B_w_i.T, *consts)
    return out.reshape(1, S, D)
```
